```python
import os as _os
_os.environ.setdefault("JAX_PLATFORMS", "cpu")
import jax
import jax.numpy as jnp

def _softmax(x, axis=-1):
    return jax.nn.softmax(x, axis=axis)
def _gelu(x):
    return jax.nn.gelu(x, approximate=True)
def _silu(x):
    return jax.nn.silu(x)
def _sigmoid(x):
    return jax.nn.sigmoid(x)
def _layernorm(x, axis=-1, eps=1e-5):
    m = jnp.mean(x, axis=axis, keepdims=True)
    v = jnp.var(x, axis=axis, keepdims=True)
    return (x - m) / jnp.sqrt(v + eps)
def _scatter_add(tgt, idx, src, axis=0):
    return tgt.at[idx].add(src)
def _segment_sum(src, seg, n):
    return jax.ops.segment_sum(src, seg, n)
class _Rng:
    def __init__(self, key):
        self._k = key
    def _next(self):
        self._k, sub = jax.random.split(self._k)
        return sub
    def normal(self, shape):
        return jax.random.normal(self._next(), shape, dtype=jnp.bfloat16)
    def randint(self, lo, hi, shape):
        return jax.random.randint(self._next(), shape, lo, hi, dtype=jnp.int32)
    def uniform(self, shape, lo=0.0, hi=1.0):
        return jax.random.uniform(self._next(), shape, jnp.bfloat16, lo, hi)
    def permutation(self, n):
        return jax.random.permutation(self._next(), n)


kernel_name = 'sequential_preLN__softmax_full_mha__dense_activation_gelu__prompt'

def setup_inputs():
    _rng = _Rng(jax.random.key(int.from_bytes(__import__("os").urandom(4), "little")))
    _w = (lambda a: (lambda t: t.astype(jnp.bfloat16) if jnp.issubdtype(t.dtype, jnp.floating) else t)(jnp.asarray(a)))
    def _A_setup():
        B, S, D = 1, 2048, 512
        return {
            "x": _w((lambda *s: _rng.normal(s) * 0.05)(B, S, D)),
            "wqkv": _w((lambda *s: _rng.normal(s) * 0.05)(D, 3 * D)),
            "wo": _w((lambda *s: _rng.normal(s) * 0.05)(D, D)),
        }
    _A_in = _A_setup()

    def _B_setup():
        B, S, D, F = 1, 2048, 512, 1792
        return {
            "x": _w((lambda *s: _rng.normal(s) * 0.05)(B, S, D)),
            "w1": _w((lambda *s: _rng.normal(s) * 0.4)(D, F) * (D ** -0.5)),
            "b1": _w((lambda *s: _rng.normal(s) * 0.4)(F) * 0.01),
            "w2": _w((lambda *s: _rng.normal(s) * 0.4)(F, D) * (F ** -0.5)),
            "b2": _w((lambda *s: _rng.normal(s) * 0.05)(D) * 0.01),
        }
    _B_in = _B_setup()

    return {
        "A_x": _A_in["x"],
        "A_wqkv": _A_in["wqkv"],
        "A_wo": _A_in["wo"],
        "B_x": _B_in["x"],
        "B_w1": _B_in["w1"],
        "B_b1": _B_in["b1"],
        "B_w2": _B_in["w2"],
        "B_b2": _B_in["b2"],
    }

def reference(A_x, A_wqkv, A_wo, B_x, B_w1, B_b1, B_w2, B_b2):
    def _A_ref(x, wqkv, wo):
        B, S, D = x.shape
        H = 32; Dh = D // H
        qkv = (lambda x, *d: x.transpose(*d))((x @ wqkv).reshape(B, S, 3, H, Dh), 2, 0, 3, 1, 4)
        q, k, v = qkv[0], qkv[1], qkv[2]
        scale = Dh ** -0.5
        scores = jnp.einsum("bhqd,bhkd->bhqk", q, k) * scale
        p = _softmax(scores, axis=-1)
        o = jnp.einsum("bhqk,bhkd->bhqd", p, v)
        return (lambda x, *d: x.transpose(*d))(o, 0, 2, 1, 3).reshape(B, S, D) @ wo

    def _B_ref(x, w1, b1, w2, b2):
        h = jnp.einsum("bsd,df->bsf", x, w1) + b1
        h = _gelu(h)
        return jnp.einsum("bsf,fd->bsd", h, w2) + b2

    x = A_x
    h = x + _A_ref(_layernorm(x, axis=-1), A_wqkv, A_wo)
    h2 = h + _B_ref(_layernorm(h, axis=-1), B_w1, B_b1, B_w2, B_b2)
    return h2
```

```python
import functools
import math

import jax
import jax.numpy as jnp
from jax import lax
import jax.experimental.pallas as pl
import jax.experimental.pallas.tpu as pltpu

_H = 32
_EPS = 1e-5
_TB = 512
_TQ = 512
_CK = 128


def _layernorm(x):
    m = jnp.mean(x, axis=-1, keepdims=True)
    xc = x - m
    v = jnp.mean(xc * xc, axis=-1, keepdims=True)
    return xc * lax.rsqrt(v + _EPS)


def _gelu_tanh(x):
    c = math.sqrt(2.0 / math.pi)
    inner = x * (c + (c * 0.044715) * (x * x))
    hx = 0.5 * x
    return hx + hx * jnp.tanh(inner)


def _kernel(x_ref, wqkv_ref, wo_ref, w1_ref, b1_ref, w2_ref, b2_ref, o_ref,
            wqvt_scr, kh_scr, qt_scr, vt_scr, ot_scr, s_a, s_b, m_scr,
            *, S, D, F):
    H = _H
    Dh = D // H
    HPG = 128 // Dh
    NG = D // 128
    TB, TQ, CK = _TB, _TQ, _CK
    NQ = S // TQ
    NC = S // CK
    NU = H * NQ
    f32 = jnp.float32
    bf16 = jnp.bfloat16
    qscale = (Dh ** -0.5) * math.log2(math.e)

    wqvt_scr[0:D, :] = wqkv_ref[:, 0:D].T
    wqvt_scr[D:2 * D, :] = wqkv_ref[:, 2 * D:3 * D].T

    def p1(b, carry):
        r0 = pl.multiple_of(b * TB, TB)
        xn = _layernorm(x_ref[pl.ds(r0, TB), :].astype(f32)).astype(bf16)
        qv = lax.dot_general(wqvt_scr[...], xn, (((1,), (1,)), ((), ())),
                             preferred_element_type=f32)
        qt_scr[:, pl.ds(r0, TB)] = (qv[0:D] * qscale).astype(bf16)
        vt_scr[:, pl.ds(r0, TB)] = qv[D:2 * D].astype(bf16)
        k = jnp.dot(xn, wqkv_ref[:, D:2 * D], preferred_element_type=f32)
        kb = pltpu.bitcast(k.astype(bf16), jnp.uint32)
        for g in range(NG):
            kg = kb[:, g * 128:(g + 1) * 128]
            for j in range(HPG):
                kr = kg if j == 0 else pltpu.roll(kg, 128 - j * Dh, axis=1)
                kh_scr[g * HPG + j, pl.ds(r0, TB), :] = pltpu.bitcast(kr, bf16)
        return carry

    lax.fori_loop(0, S // TB, p1, 0)

    def pass1_chunk(u, s_scr, c, m):
        h = u // NQ
        qb = u % NQ
        kc = kh_scr[h, pl.ds(c * CK, CK), 0:Dh]
        qt = qt_scr[pl.ds(pl.multiple_of(h * Dh, Dh), Dh),
                    pl.ds(pl.multiple_of(qb * TQ, TQ), TQ)]
        s = jnp.dot(kc, qt, preferred_element_type=f32)
        s_scr[pl.ds(c * CK, CK), :] = s
        return jnp.maximum(m, jnp.max(s.reshape(CK // 8, 8, TQ), axis=0))

    def pass2_chunk(u, s_scr, c, m, l, o):
        h = u // NQ
        p = jnp.exp2(s_scr[pl.ds(c * CK, CK), :] - m)
        l = l + jnp.sum(p.reshape(CK // 8, 8, TQ), axis=0)
        vt = vt_scr[pl.ds(pl.multiple_of(h * Dh, Dh), Dh), pl.ds(c * CK, CK)]
        o = o + jnp.dot(vt, p.astype(bf16), preferred_element_type=f32)
        return l, o

    def finish(u, l, o):
        h = u // NQ
        qb = u % NQ
        lt = jnp.sum(l, axis=0, keepdims=True)
        ot_scr[pl.ds(pl.multiple_of(h * Dh, Dh), Dh),
               pl.ds(pl.multiple_of(qb * TQ, TQ), TQ)] = (o / lt).astype(bf16)

    neg = jnp.full((8, TQ), -jnp.inf, f32)

    def step(u, s_cur, s_nxt, do1, do2):
        m = neg
        if do2:
            mprev = m_scr[...]
            l = jnp.zeros((8, TQ), f32)
            o = jnp.zeros((Dh, TQ), f32)
        for c in range(NC):
            if do1:
                m = pass1_chunk(u + 1, s_nxt, c, m)
            if do2:
                l, o = pass2_chunk(u, s_cur, c, mprev, l, o)
        if do2:
            finish(u, l, o)
        if do1:
            m_scr[...] = jnp.max(m, axis=0, keepdims=True)

    step(-1, None, s_a, True, False)

    def body(u, carry):
        @pl.when(u % 2 == 0)
        def _():
            step(u, s_a, s_b, True, True)

        @pl.when(u % 2 == 1)
        def _():
            step(u, s_b, s_a, True, True)
        return carry

    lax.fori_loop(0, NU - 1, body, 0)
    step(NU - 1, s_b if (NU - 1) % 2 else s_a, None, False, True)

    def p3(b, carry):
        r0 = pl.multiple_of(b * TB, TB)
        attn = lax.dot_general(ot_scr[:, pl.ds(r0, TB)], wo_ref[...],
                               (((0,), (0,)), ((), ())),
                               preferred_element_type=f32)
        h = x_ref[pl.ds(r0, TB), :].astype(f32) + attn
        hn = _layernorm(h).astype(bf16)
        a = jnp.dot(hn, w1_ref[...], preferred_element_type=f32) + b1_ref[...].astype(f32)
        g = _gelu_tanh(a).astype(bf16)
        y = jnp.dot(g, w2_ref[...], preferred_element_type=f32) + b2_ref[...].astype(f32)
        o_ref[pl.ds(r0, TB), :] = (h + y).astype(o_ref.dtype)
        return carry

    lax.fori_loop(0, S // TB, p3, 0)


@jax.jit
def pallas_sequential_preLN__softmax_full_mha__dense_activation_gelu__prompt_kernel(
    A_x: jax.Array,
    A_wqkv: jax.Array,
    A_wo: jax.Array,
    B_x: jax.Array,
    B_w1: jax.Array,
    B_b1: jax.Array,
    B_w2: jax.Array,
    B_b2: jax.Array,
):
    B, S, D = A_x.shape
    F = B_w1.shape[1]
    assert B == 1
    bf16 = jnp.bfloat16
    f32 = jnp.float32
    out = pl.pallas_call(
        functools.partial(_kernel, S=S, D=D, F=F),
        out_shape=jax.ShapeDtypeStruct((S, D), A_x.dtype),
        scratch_shapes=[
            pltpu.VMEM((2 * D, D), bf16),
            pltpu.VMEM((_H, S, 128), bf16),
            pltpu.VMEM((D, S), bf16),
            pltpu.VMEM((D, S), bf16),
            pltpu.VMEM((D, S), bf16),
            pltpu.VMEM((S, _TQ), f32),
            pltpu.VMEM((S, _TQ), f32),
            pltpu.VMEM((1, _TQ), f32),
        ],
        compiler_params=pltpu.CompilerParams(vmem_limit_bytes=100 * 1024 * 1024),
    )(A_x.reshape(S, D), A_wqkv, A_wo, B_w1, B_b1.reshape(1, F), B_w2,
      B_b2.reshape(1, D))
    return out.reshape(B, S, D)
```

```python
import functools
import math

import jax
import jax.numpy as jnp
from jax import lax
import jax.experimental.pallas as pl
import jax.experimental.pallas.tpu as pltpu

_H = 32
_EPS = 1e-5
_SB1 = 256
_TQ = 512
_CK = 128
_EXTRA = 2
_NV = 14
_HB = 2
_HP = 2
_DM = 4
_DV = 3
_DK = 4
_QD = 3
_KBSTEPS = (4, 10)
_QSTEPS = (14, 15)
_P3_BOUNDS = (0, 256, 512, 768, 1024, 1280, 1536, 1792, 1920, 2048)
_B2_OFF = 4096


def _layernorm(x):
    m = jnp.mean(x, axis=-1, keepdims=True)
    xc = x - m
    v = jnp.mean(xc * xc, axis=-1, keepdims=True)
    return xc * lax.rsqrt(v + _EPS)


def _gelu_tanh(x):
    c = math.sqrt(2.0 / math.pi)
    inner = x * (c + (c * 0.044715) * (x * x))
    hx = 0.5 * x
    return hx + hx * jnp.tanh(inner)


def _kernel(x_hbm, wqkv_hbm, wo_hbm, w1_hbm, b1_hbm, w2_hbm, b2_hbm, o_hbm,
            x_ref, wqkv_ref, wo_ref, w1_ref, w2_ref, o_ref,
            wqvt_scr, kh_scr, qt_scr, vt_scr, ot_scr, s0, s1, s2, s3,
            kb0, kb1, qb_scr, m_scr, l_scr, acc_scr, z_scr, b_ref,
            x_sem, w_sem, o_sem, f_sem,
            *, S, D, F):
    H = _H
    Dh = D // H
    HPG = 128 // Dh
    NG = D // 128
    TQ, CK, SB1 = _TQ, _CK, _SB1
    NQ = S // TQ
    NC = S // CK
    LAG = NC + _EXTRA
    f32 = jnp.float32
    bf16 = jnp.bfloat16
    u32 = jnp.uint32
    qscale = (Dh ** -0.5) * math.log2(math.e)
    sb = [s0, s1, s2, s3]
    kb_scr = [kb0, kb1]
    assert NQ == len(sb)

    XS = 2 * SB1

    def x_copy(i, r0, r1):
        return pltpu.make_async_copy(x_hbm.at[r0:r1, :], x_ref.at[r0:r1, :],
                                     x_sem.at[i])

    def wqkv_copy(i):
        return pltpu.make_async_copy(wqkv_hbm.at[:, i * D:(i + 1) * D],
                                     wqkv_ref.at[i], w_sem.at[i])

    xa_copy = x_copy(0, 0, XS)
    xb_copy = x_copy(1, XS, 2 * XS)
    xc_copy = x_copy(2, 2 * XS, S)
    late_copies = [
        pltpu.make_async_copy(wo_hbm, wo_ref, w_sem.at[3]),
        pltpu.make_async_copy(w1_hbm, w1_ref, w_sem.at[4]),
        pltpu.make_async_copy(w2_hbm, w2_ref, w_sem.at[5]),
        pltpu.make_async_copy(b1_hbm, b_ref.at[0:F], w_sem.at[6]),
        pltpu.make_async_copy(b2_hbm, b_ref.at[_B2_OFF:_B2_OFF + D], w_sem.at[7]),
    ]

    for cp in (xa_copy, wqkv_copy(1), wqkv_copy(0), wqkv_copy(2), xb_copy, xc_copy):
        cp.start()
        pl.semaphore_signal(f_sem, 1)
        pl.semaphore_wait(f_sem, 1)
    z_scr[...] = jnp.zeros(z_scr.shape, u32)

    N1 = S // SB1
    xn = [None] * N1
    kp = [None] * N1

    def ln1(i):
        xn[i] = _layernorm(x_ref[i * SB1:(i + 1) * SB1, :].astype(f32)).astype(bf16)

    def kmm(i):
        k = jnp.dot(xn[i], wqkv_ref[1], preferred_element_type=f32)
        kp[i] = pltpu.bitcast(k.astype(bf16), u32)

    def kstore(i):
        for g in range(NG):
            kg = kp[i][:, g * 128:(g + 1) * 128]
            for j in range(HPG):
                kr = kg if j == 0 else pltpu.roll(kg, 128 - j * Dh, axis=1)
                kh_scr[g * HPG + j, i * (SB1 // 2):(i + 1) * (SB1 // 2), :] = kr

    def qnat(i):
        q = jnp.dot(xn[i], wqkv_ref[0], preferred_element_type=f32)
        return (q * qscale).astype(bf16)

    def vnat(i):
        v = jnp.dot(xn[i], wqkv_ref[2], preferred_element_type=f32)
        return v.astype(bf16)

    def tstore(dst, i, val):
        dst[:, i * SB1:(i + 1) * SB1] = val.T

    def qvproj(i):
        qv = lax.dot_general(wqvt_scr[...], xn[i], (((1,), (1,)), ((), ())),
                             preferred_element_type=f32)
        qt_scr[:, i * SB1:(i + 1) * SB1] = (qv[0:D] * qscale).astype(bf16)
        vt_scr[:, i * SB1:(i + 1) * SB1] = qv[D:2 * D].astype(bf16)

    xa_copy.wait()
    ln1(0)
    ln1(1)
    wqkv_copy(1).wait()
    kmm(0)
    kmm(1)
    wqkv_copy(0).wait()
    q0 = qnat(0)
    wqvt_scr[0:D, :] = wqkv_ref[0].T
    q1 = qnat(1)
    tstore(qt_scr, 0, q0)
    wqkv_copy(2).wait()
    xb_copy.wait()
    v0 = vnat(0)
    wqvt_scr[D:2 * D, :] = wqkv_ref[2].T
    v1 = vnat(1)
    ln1(2)
    tstore(qt_scr, 1, q1)
    tstore(vt_scr, 0, v0)
    tstore(vt_scr, 1, v1)
    kstore(0)
    for i in range(2, N1):
        kmm(i)
        if i == 3:
            xc_copy.wait()
        if i + 1 < N1:
            ln1(i + 1)
        qvproj(i)
        kstore(i - 1)
    kstore(N1 - 1)

    T = NQ * NC
    NV = _NV
    KV = 8 * NV
    hi = [KV + (((S - KV) // 16) * (c + 1)) // NC * 16 for c in range(NC)]
    lo = [KV] + hi[:-1]
    assert hi[-1] == S and KV % 16 == 0 and NV <= NC
    NJ = TQ // 128

    def head_rows(h):
        return pl.ds(pl.multiple_of(h * Dh, Dh), Dh)

    def gen_kb(h, kb_ref, ds):
        kf = pltpu.bitcast(kh_scr[h, 0:KV // 2, :], bf16).astype(f32)
        for d in ds:
            kbc = jnp.broadcast_to(kf[:, d:d + 1], (KV, 128))
            kb_ref[d] = kbc
        return kbc[KV - 8:]

    def gen_qb(h, u, ds):
        qf = qt_scr[head_rows(h), (u % NQ) * TQ:(u % NQ + 1) * TQ].astype(f32)
        for d in ds:
            qbc = jnp.broadcast_to(qf[d:d + 1, :], (8, TQ))
            qb_scr[u % qb_scr.shape[0], d] = qbc
        return qbc[:, TQ - 128:]

    def run(h0, n_steps, do1, do2, hook=None, first=False):
        z = jnp.concatenate([z_scr[0:8, :]] * NJ, axis=1)
        m = None
        st = None
        mh = []
        gdep = []
        for t in range(n_steps):
            if do1(t):
                h = h0 + t // T
                u = t // NC
                qb, c = divmod(t % T, NC)
                if first and t == 0:
                    gen_kb(h0, kb_scr[0], range(Dh))
                    gen_qb(h0, 0, range(Dh))
                if c in _QSTEPS:
                    n = _QSTEPS.index(c)
                    hq = h0 + (u + 1) // NQ
                    if (u + 1) * NC >= n_steps:
                        hq = jnp.minimum(hq, H - 1)
                    last = gen_qb(hq, u + 1, range(n * Dh // len(_QSTEPS),
                                                   (n + 1) * Dh // len(_QSTEPS)))
                    gdep.append((t + _QD, last))
                kc = pltpu.bitcast(
                    kh_scr[h, pl.ds(lo[c] // 2, (hi[c] - lo[c]) // 2), :],
                    bf16)[:, 0:Dh]
                qt = qt_scr[head_rows(h), qb * TQ:(qb + 1) * TQ]
                s = jnp.dot(kc, qt, preferred_element_type=f32)
                sb[qb][pl.ds(lo[c], hi[c] - lo[c]), :] = s
                mc = jnp.max(s.reshape((hi[c] - lo[c]) // 8, 8, TQ), axis=0)
                m = mc if c == 0 else jnp.maximum(m, mc)
                mh.append(m)
                if c < NV:
                    acc = None
                    for d in range(Dh):
                        kbv = kb_scr[(t // T) % 2][d, pl.ds(c * 8, 8), :]
                        if len(mh) >= _DV:
                            depz = pltpu.bitcast(mh[-_DV][:, 0:128], u32) & z[:, 0:128]
                            kbv = pltpu.bitcast(pltpu.bitcast(kbv, u32) | depz, f32)
                        pr = (jnp.concatenate([kbv] * NJ, axis=1)
                              * qb_scr[u % qb_scr.shape[0], d])
                        acc = pr if acc is None else acc + pr
                    sb[qb][pl.ds(c * 8, 8), :] = acc
                    m = jnp.maximum(m, acc)
                if c == NC - 1:
                    m_scr[qb] = jnp.broadcast_to(
                        jnp.max(m, axis=0, keepdims=True), (8, TQ))
                if c in _KBSTEPS:
                    nslot = NQ * len(_KBSTEPS)
                    slot = qb * len(_KBSTEPS) + _KBSTEPS.index(c)
                    last = gen_kb(jnp.minimum(h + 1, H - 1),
                                  kb_scr[(t // T + 1) % 2],
                                  range(slot * Dh // nslot, (slot + 1) * Dh // nslot))
                    gdep.append((t + _DK, last))
                gdep.sort(key=lambda e: e[0])
            t2 = t - LAG
            if do2(t2):
                h2 = h0 + t2 // T
                qb, c = divmod(t2 % T, NC)
                if c == 0:
                    st = (m_scr[qb], jnp.zeros((8, TQ), f32),
                          jnp.zeros((Dh, TQ), f32))
                elif st is None:
                    st = (m_scr[qb], l_scr[...], acc_scr[...])
                mm, l, o = st
                mu = mm
                if len(mh) >= _DM:
                    dep = mh[-_DM]
                    if gdep and t >= gdep[0][0]:
                        dep = jnp.concatenate(
                            [dep[:, 0:128] + gdep.pop(0)[1], dep[:, 128:]], axis=1)
                    mu = pltpu.bitcast(
                        pltpu.bitcast(mm, u32) | (pltpu.bitcast(dep, u32) & z), f32)
                sc = sb[qb][pl.ds(c * CK, CK), :].reshape(CK // 8, 8, TQ)
                p = jnp.exp2(sc - mu[None])
                for i in reversed(range(CK // 16)):
                    l = l + (p[2 * i + 1] + p[2 * i])
                vt = vt_scr[head_rows(h2), pl.ds(c * CK, CK)]
                o = o + jnp.dot(vt, p.reshape(CK, TQ).astype(bf16),
                                preferred_element_type=f32)
                st = (mm, l, o)
                if c == NC - 1:
                    lt = jnp.sum(l, axis=0, keepdims=True)
                    ot_scr[head_rows(h2), qb * TQ:(qb + 1) * TQ] = (o / lt).astype(bf16)
                    st = None
            if hook is not None:
                hook(t)
        if st is not None:
            l_scr[...] = st[1]
            acc_scr[...] = st[2]

    assert (H - _HP) % _HB == 0 and _HP % 2 == 0 and _HB % 2 == 0
    run(0, _HP * T, lambda t: True, lambda t2: t2 >= 0, first=True)
    for cp in late_copies:
        cp.start()

    def body(i, carry):
        run(_HP + i * _HB, _HB * T, lambda t: True, lambda t2: True)
        return carry

    lax.fori_loop(0, (H - _HP) // _HB, body, 0)
    for cp in late_copies:
        cp.wait()

    bounds = _P3_BOUNDS
    NS = len(bounds) - 1
    rows = [pl.ds(bounds[i], bounds[i + 1] - bounds[i]) for i in range(NS)]
    hs = [None] * NS
    gs = [None] * NS
    b1 = b_ref[0:F].astype(f32).reshape(1, F)
    b2 = b_ref[_B2_OFF:_B2_OFF + D].astype(f32).reshape(1, D)

    def o_copy(i):
        return pltpu.make_async_copy(o_ref.at[rows[i], :], o_hbm.at[rows[i], :],
                                     o_sem.at[i])

    def op(i):
        attn = lax.dot_general(ot_scr[:, rows[i]], wo_ref[...],
                               (((0,), (0,)), ((), ())),
                               preferred_element_type=f32)
        hs[i] = x_ref[rows[i], :].astype(f32) + attn

    def f1(i):
        hn = _layernorm(hs[i]).astype(bf16)
        a = jnp.dot(hn, w1_ref[...], preferred_element_type=f32)
        gs[i] = _gelu_tanh(a + b1).astype(bf16)

    def f2(i):
        y = jnp.dot(gs[i], w2_ref[...], preferred_element_type=f32)
        o_ref[rows[i], :] = (hs[i] + (y + b2)).astype(o_ref.dtype)
        o_copy(i).start()

    assert bounds[2] <= TQ
    pieces = {}
    ob = [ot_scr[:, rows[i]].T for i in range(2)]

    def hook(t):
        n = ((t + 1) * 2 * NG) // LAG - (t * 2 * NG) // LAG
        for _ in range(n):
            i, g = divmod(len(pieces), NG)
            pieces[(i, g)] = jnp.dot(ob[i], wo_ref[:, g * 128:(g + 1) * 128],
                                     preferred_element_type=f32)

    run(H, LAG, lambda t: False, lambda t2: True, hook)
    for i in range(2):
        attn = jnp.concatenate([pieces[(i, g)] for g in range(NG)], axis=1)
        hs[i] = x_ref[rows[i], :].astype(f32) + attn
    for i in range(NS):
        f1(i)
        if i + 2 < NS:
            op(i + 2)
        if i >= 1:
            f2(i - 1)
    f2(NS - 1)
    for i in range(NS):
        o_copy(i).wait()


@jax.jit
def pallas_sequential_preLN__softmax_full_mha__dense_activation_gelu__prompt_kernel(
    A_x: jax.Array,
    A_wqkv: jax.Array,
    A_wo: jax.Array,
    B_x: jax.Array,
    B_w1: jax.Array,
    B_b1: jax.Array,
    B_w2: jax.Array,
    B_b2: jax.Array,
):
    del B_x
    B, S, D = A_x.shape
    F = B_w1.shape[1]
    assert B == 1 and S == _P3_BOUNDS[-1] and F <= _B2_OFF
    bf16 = jnp.bfloat16
    f32 = jnp.float32
    nq = S // _TQ
    dh = D // _H
    hbm = pl.BlockSpec(memory_space=pl.ANY)
    out = pl.pallas_call(
        functools.partial(_kernel, S=S, D=D, F=F),
        out_shape=jax.ShapeDtypeStruct((S, D), A_x.dtype),
        in_specs=[hbm] * 7,
        out_specs=hbm,
        scratch_shapes=[
            pltpu.VMEM((S, D), bf16),
            pltpu.VMEM((3, D, D), bf16),
            pltpu.VMEM((D, D), bf16),
            pltpu.VMEM((D, F), bf16),
            pltpu.VMEM((F, D), bf16),
            pltpu.VMEM((S, D), A_x.dtype),
            pltpu.VMEM((2 * D, D), bf16),
            pltpu.VMEM((_H, S // 2, 128), jnp.uint32),
            pltpu.VMEM((D, S), bf16),
            pltpu.VMEM((D, S), bf16),
            pltpu.VMEM((D, S), bf16),
        ] + [pltpu.VMEM((S, _TQ), f32)] * nq + [
            pltpu.VMEM((dh, 8 * _NV, 128), f32),
            pltpu.VMEM((dh, 8 * _NV, 128), f32),
            pltpu.VMEM((_HB * nq, dh, 8, _TQ), f32),
            pltpu.VMEM((nq, 8, _TQ), f32),
            pltpu.VMEM((8, _TQ), f32),
            pltpu.VMEM((dh, _TQ), f32),
            pltpu.VMEM((32, 128), jnp.uint32),
            pltpu.VMEM((2 * _B2_OFF,), bf16),
            pltpu.SemaphoreType.DMA((3,)),
            pltpu.SemaphoreType.DMA((8,)),
            pltpu.SemaphoreType.DMA((len(_P3_BOUNDS) - 1,)),
            pltpu.SemaphoreType.REGULAR,
        ],
        compiler_params=pltpu.CompilerParams(vmem_limit_bytes=100 * 1024 * 1024),
    )(A_x.reshape(S, D), A_wqkv, A_wo, B_w1, B_b1, B_w2, B_b2)
    return out.reshape(B, S, D)
```

```python
import functools
import math

import jax
import jax.numpy as jnp
from jax import lax
import jax.experimental.pallas as pl
import jax.experimental.pallas.tpu as pltpu

_H = 32
_EPS = 1e-5
_SB1 = 256
_TQ = 512
_CK = 128
_EXTRA = 2
_NV = 14
_HB = 2
_HP = 2
_DM = 4
_DV = 3
_DK = 4
_QD = 3
_KBSTEPS = (4, 10)
_QSTEPS = (14, 15)
_P3_BOUNDS = (0, 256, 512, 768, 1024, 1280, 1536, 1792, 1920, 2048)
_NI = 3
_B2_OFF = 4096


def _layernorm(x):
    m = jnp.mean(x, axis=-1, keepdims=True)
    xc = x - m
    v = jnp.mean(xc * xc, axis=-1, keepdims=True)
    return xc * lax.rsqrt(v + _EPS)


def _gelu_tanh(x):
    c = math.sqrt(2.0 / math.pi)
    inner = x * (c + (c * 0.044715) * (x * x))
    hx = 0.5 * x
    return hx + hx * jnp.tanh(inner)


def _kernel(x_hbm, wqkv_hbm, wo_hbm, w1_hbm, b1_hbm, w2_hbm, b2_hbm, o_hbm,
            x_ref, wqkv_ref, wo_ref, w1_ref, w2_ref, o_ref,
            wqvt_scr, kh_scr, qt_scr, vt_scr, ot_scr, s0, s1, s2, s3,
            kb0, kb1, qb_scr, m_scr, l_scr, acc_scr, z_scr, b_ref,
            sems, f_sem,
            *, S, D, F):
    H = _H
    Dh = D // H
    HPG = 128 // Dh
    NG = D // 128
    TQ, CK, SB1 = _TQ, _CK, _SB1
    NQ = S // TQ
    NC = S // CK
    LAG = NC + _EXTRA
    f32 = jnp.float32
    bf16 = jnp.bfloat16
    u32 = jnp.uint32
    qscale = (Dh ** -0.5) * math.log2(math.e)
    sb = [s0, s1, s2, s3]
    kb_scr = [kb0, kb1]
    assert NQ == len(sb)

    XS = 2 * SB1

    def x_copy(i, r0, r1):
        return pltpu.make_async_copy(x_hbm.at[r0:r1, :], x_ref.at[r0:r1, :],
                                     sems.at[3 + i])

    def wqkv_copy(i):
        return pltpu.make_async_copy(wqkv_hbm.at[:, i * D:(i + 1) * D],
                                     wqkv_ref.at[i], sems.at[i])

    xa_copy = x_copy(0, 0, XS)
    xb_copy = x_copy(1, XS, 2 * XS)
    xc_copy = x_copy(2, 2 * XS, S)
    late_copies = [
        pltpu.make_async_copy(wo_hbm, wo_ref, sems.at[0]),
        pltpu.make_async_copy(w1_hbm, w1_ref, sems.at[0]),
        pltpu.make_async_copy(w2_hbm, w2_ref, sems.at[0]),
        pltpu.make_async_copy(b1_hbm, b_ref.at[0:F], sems.at[0]),
        pltpu.make_async_copy(b2_hbm, b_ref.at[_B2_OFF:_B2_OFF + D], sems.at[0]),
    ]

    def fence():
        pl.semaphore_signal(f_sem, 1)
        pl.semaphore_wait(f_sem, 1)

    for cp in (xa_copy, wqkv_copy(1), wqkv_copy(0), wqkv_copy(2), xb_copy, xc_copy):
        cp.start()
        fence()
    z_scr[...] = jnp.zeros(z_scr.shape, u32)

    N1 = S // SB1
    xn = [None] * N1
    kp = [None] * N1

    def ln1(i):
        xn[i] = _layernorm(x_ref[i * SB1:(i + 1) * SB1, :].astype(f32)).astype(bf16)

    def kmm(i):
        k = jnp.dot(xn[i], wqkv_ref[1], preferred_element_type=f32)
        kp[i] = pltpu.bitcast(k.astype(bf16), u32)

    def kstore(i):
        for g in range(NG):
            kg = kp[i][:, g * 128:(g + 1) * 128]
            for j in range(HPG):
                kr = kg if j == 0 else pltpu.roll(kg, 128 - j * Dh, axis=1)
                kh_scr[g * HPG + j, i * (SB1 // 2):(i + 1) * (SB1 // 2), :] = kr

    def qnat(i):
        q = jnp.dot(xn[i], wqkv_ref[0], preferred_element_type=f32)
        return (q * qscale).astype(bf16)

    def vnat(i):
        v = jnp.dot(xn[i], wqkv_ref[2], preferred_element_type=f32)
        return v.astype(bf16)

    def tstore(dst, i, val):
        dst[:, i * SB1:(i + 1) * SB1] = val.T

    def qvproj(i):
        qv = lax.dot_general(wqvt_scr[...], xn[i], (((1,), (1,)), ((), ())),
                             preferred_element_type=f32)
        qt_scr[:, i * SB1:(i + 1) * SB1] = (qv[0:D] * qscale).astype(bf16)
        vt_scr[:, i * SB1:(i + 1) * SB1] = qv[D:2 * D].astype(bf16)

    xa_copy.wait()
    ln1(0)
    ln1(1)
    wqkv_copy(1).wait()
    kmm(0)
    kmm(1)
    wqkv_copy(0).wait()
    q0 = qnat(0)
    wqvt_scr[0:D, :] = wqkv_ref[0].T
    q1 = qnat(1)
    tstore(qt_scr, 0, q0)
    wqkv_copy(2).wait()
    xb_copy.wait()
    v0 = vnat(0)
    wqvt_scr[D:2 * D, :] = wqkv_ref[2].T
    v1 = vnat(1)
    ln1(2)
    tstore(qt_scr, 1, q1)
    tstore(vt_scr, 0, v0)
    tstore(vt_scr, 1, v1)
    kstore(0)
    for i in range(2, N1):
        kmm(i)
        if i == 3:
            xc_copy.wait()
        if i + 1 < N1:
            ln1(i + 1)
        qvproj(i)
        kstore(i - 1)
    kstore(N1 - 1)

    T = NQ * NC
    NV = _NV
    KV = 8 * NV
    hi = [KV + (((S - KV) // 16) * (c + 1)) // NC * 16 for c in range(NC)]
    lo = [KV] + hi[:-1]
    assert hi[-1] == S and KV % 16 == 0 and NV <= NC
    NJ = TQ // 128

    def head_rows(h):
        return pl.ds(pl.multiple_of(h * Dh, Dh), Dh)

    def gen_kb(h, kb_ref, ds):
        kf = pltpu.bitcast(kh_scr[h, 0:KV // 2, :], bf16).astype(f32)
        for d in ds:
            kbc = jnp.broadcast_to(kf[:, d:d + 1], (KV, 128))
            kb_ref[d] = kbc
        return kbc[KV - 8:]

    def gen_qb(h, u, ds):
        qf = qt_scr[head_rows(h), (u % NQ) * TQ:(u % NQ + 1) * TQ].astype(f32)
        for d in ds:
            qbc = jnp.broadcast_to(qf[d:d + 1, :], (8, TQ))
            qb_scr[u % qb_scr.shape[0], d] = qbc
        return qbc[:, TQ - 128:]

    def run(h0, n_steps, do1, do2, hook=None, first=False):
        z = jnp.concatenate([z_scr[0:8, :]] * NJ, axis=1)
        m = None
        st = None
        mh = []
        gdep = []
        for t in range(n_steps):
            if do1(t):
                h = h0 + t // T
                u = t // NC
                qb, c = divmod(t % T, NC)
                if first and t == 0:
                    gen_kb(h0, kb_scr[0], range(Dh))
                    gen_qb(h0, 0, range(Dh))
                if c in _QSTEPS:
                    n = _QSTEPS.index(c)
                    hq = h0 + (u + 1) // NQ
                    if (u + 1) * NC >= n_steps:
                        hq = jnp.minimum(hq, H - 1)
                    last = gen_qb(hq, u + 1, range(n * Dh // len(_QSTEPS),
                                                   (n + 1) * Dh // len(_QSTEPS)))
                    gdep.append((t + _QD, last))
                kc = pltpu.bitcast(
                    kh_scr[h, pl.ds(lo[c] // 2, (hi[c] - lo[c]) // 2), :],
                    bf16)[:, 0:Dh]
                qt = qt_scr[head_rows(h), qb * TQ:(qb + 1) * TQ]
                s = jnp.dot(kc, qt, preferred_element_type=f32)
                sb[qb][pl.ds(lo[c], hi[c] - lo[c]), :] = s
                mc = jnp.max(s.reshape((hi[c] - lo[c]) // 8, 8, TQ), axis=0)
                m = mc if c == 0 else jnp.maximum(m, mc)
                mh.append(m)
                if c < NV:
                    acc = None
                    for d in range(Dh):
                        kbv = kb_scr[(t // T) % 2][d, pl.ds(c * 8, 8), :]
                        if len(mh) >= _DV:
                            depz = pltpu.bitcast(mh[-_DV][:, 0:128], u32) & z[:, 0:128]
                            kbv = pltpu.bitcast(pltpu.bitcast(kbv, u32) | depz, f32)
                        pr = (jnp.concatenate([kbv] * NJ, axis=1)
                              * qb_scr[u % qb_scr.shape[0], d])
                        acc = pr if acc is None else acc + pr
                    sb[qb][pl.ds(c * 8, 8), :] = acc
                    m = jnp.maximum(m, acc)
                if c == NC - 1:
                    m_scr[qb] = jnp.broadcast_to(
                        jnp.max(m, axis=0, keepdims=True), (8, TQ))
                if c in _KBSTEPS:
                    nslot = NQ * len(_KBSTEPS)
                    slot = qb * len(_KBSTEPS) + _KBSTEPS.index(c)
                    last = gen_kb(jnp.minimum(h + 1, H - 1),
                                  kb_scr[(t // T + 1) % 2],
                                  range(slot * Dh // nslot, (slot + 1) * Dh // nslot))
                    gdep.append((t + _DK, last))
                gdep.sort(key=lambda e: e[0])
            t2 = t - LAG
            if do2(t2):
                h2 = h0 + t2 // T
                qb, c = divmod(t2 % T, NC)
                if c == 0:
                    st = (m_scr[qb], jnp.zeros((8, TQ), f32),
                          jnp.zeros((Dh, TQ), f32))
                elif st is None:
                    st = (m_scr[qb], l_scr[...], acc_scr[...])
                mm, l, o = st
                mu = mm
                if len(mh) >= _DM:
                    dep = mh[-_DM]
                    if gdep and t >= gdep[0][0]:
                        dep = jnp.concatenate(
                            [dep[:, 0:128] + gdep.pop(0)[1], dep[:, 128:]], axis=1)
                    mu = pltpu.bitcast(
                        pltpu.bitcast(mm, u32) | (pltpu.bitcast(dep, u32) & z), f32)
                sc = sb[qb][pl.ds(c * CK, CK), :].reshape(CK // 8, 8, TQ)
                p = jnp.exp2(sc - mu[None])
                for i in reversed(range(CK // 16)):
                    l = l + (p[2 * i + 1] + p[2 * i])
                vt = vt_scr[head_rows(h2), pl.ds(c * CK, CK)]
                o = o + jnp.dot(vt, p.reshape(CK, TQ).astype(bf16),
                                preferred_element_type=f32)
                st = (mm, l, o)
                if c == NC - 1:
                    lt = jnp.sum(l, axis=0, keepdims=True)
                    r = pl.reciprocal(lt, approx=True)
                    r = r * (2.0 - lt * r)
                    ot_scr[head_rows(h2), qb * TQ:(qb + 1) * TQ] = (o * r).astype(bf16)
                    st = None
            if hook is not None:
                hook(t)
        if st is not None:
            l_scr[...] = st[1]
            acc_scr[...] = st[2]

    assert (H - _HP) % _HB == 0 and _HP % 2 == 0 and _HB % 2 == 0
    run(0, _HP * T, lambda t: True, lambda t2: t2 >= 0, first=True)
    for cp in late_copies:
        cp.start()

    def body(i, carry):
        run(_HP + i * _HB, _HB * T, lambda t: True, lambda t2: True)
        return carry

    lax.fori_loop(0, (H - _HP) // _HB, body, 0)
    for cp in late_copies:
        cp.wait()

    bounds = _P3_BOUNDS
    NS = len(bounds) - 1
    rows = [pl.ds(bounds[i], bounds[i + 1] - bounds[i]) for i in range(NS)]
    hs = [None] * NS
    gs = [None] * NS
    b1 = b_ref[0:F].astype(f32).reshape(1, F)
    b2 = b_ref[_B2_OFF:_B2_OFF + D].astype(f32).reshape(1, D)

    def o_copy(i):
        return pltpu.make_async_copy(o_ref.at[rows[i], :], o_hbm.at[rows[i], :],
                                     sems.at[1])

    def op(i):
        attn = lax.dot_general(ot_scr[:, rows[i]], wo_ref[...],
                               (((0,), (0,)), ((), ())),
                               preferred_element_type=f32)
        hs[i] = x_ref[rows[i], :].astype(f32) + attn

    def f1(i, hn=None):
        if hn is None:
            hn = _layernorm(hs[i]).astype(bf16)
        a = jnp.dot(hn, w1_ref[...], preferred_element_type=f32)
        gs[i] = _gelu_tanh(a + b1).astype(bf16)

    def f2(i):
        y = jnp.dot(gs[i], w2_ref[...], preferred_element_type=f32)
        o_ref[rows[i], :] = (hs[i] + (y + b2)).astype(o_ref.dtype)
        o_copy(i).start()

    NI = _NI
    assert bounds[NI] <= ((T - LAG) // NC) * TQ
    pieces = {}
    ob = [ot_scr[:, rows[i]].T for i in range(NI)]

    def hook(t):
        for _ in range(((t + 1) * NI * NG) // LAG - len(pieces)):
            i, g = divmod(len(pieces), NG)
            pieces[(i, g)] = jnp.dot(ob[i], wo_ref[:, g * 128:(g + 1) * 128],
                                     preferred_element_type=f32)

    run(H, LAG, lambda t: False, lambda t2: True, hook)
    for i in range(NI):
        attn = jnp.concatenate([pieces[(i, g)] for g in range(NG)], axis=1)
        hs[i] = x_ref[rows[i], :].astype(f32) + attn
    hn0 = _layernorm(hs[0]).astype(bf16)
    fence()
    for i in range(NS):
        f1(i, hn0 if i == 0 else None)
        if NI <= i + 2 < NS:
            op(i + 2)
        if i >= 1:
            f2(i - 1)
    f2(NS - 1)
    for i in range(NS):
        o_copy(i).wait()


@jax.jit
def pallas_sequential_preLN__softmax_full_mha__dense_activation_gelu__prompt_kernel(
    A_x: jax.Array,
    A_wqkv: jax.Array,
    A_wo: jax.Array,
    B_x: jax.Array,
    B_w1: jax.Array,
    B_b1: jax.Array,
    B_w2: jax.Array,
    B_b2: jax.Array,
):
    del B_x
    B, S, D = A_x.shape
    F = B_w1.shape[1]
    assert B == 1 and S == _P3_BOUNDS[-1] and F <= _B2_OFF
    bf16 = jnp.bfloat16
    f32 = jnp.float32
    nq = S // _TQ
    dh = D // _H
    hbm = pl.BlockSpec(memory_space=pl.ANY)
    out = pl.pallas_call(
        functools.partial(_kernel, S=S, D=D, F=F),
        out_shape=jax.ShapeDtypeStruct((S, D), A_x.dtype),
        in_specs=[hbm] * 7,
        out_specs=hbm,
        scratch_shapes=[
            pltpu.VMEM((S, D), bf16),
            pltpu.VMEM((3, D, D), bf16),
            pltpu.VMEM((D, D), bf16),
            pltpu.VMEM((D, F), bf16),
            pltpu.VMEM((F, D), bf16),
            pltpu.VMEM((S, D), A_x.dtype),
            pltpu.VMEM((2 * D, D), bf16),
            pltpu.VMEM((_H, S // 2, 128), jnp.uint32),
            pltpu.VMEM((D, S), bf16),
            pltpu.VMEM((D, S), bf16),
            pltpu.VMEM((D, S), bf16),
        ] + [pltpu.VMEM((S, _TQ), f32)] * nq + [
            pltpu.VMEM((dh, 8 * _NV, 128), f32),
            pltpu.VMEM((dh, 8 * _NV, 128), f32),
            pltpu.VMEM((_HB * nq, dh, 8, _TQ), f32),
            pltpu.VMEM((nq, 8, _TQ), f32),
            pltpu.VMEM((8, _TQ), f32),
            pltpu.VMEM((dh, _TQ), f32),
            pltpu.VMEM((32, 128), jnp.uint32),
            pltpu.VMEM((2 * _B2_OFF,), bf16),
            pltpu.SemaphoreType.DMA((6,)),
            pltpu.SemaphoreType.REGULAR,
        ],
        compiler_params=pltpu.CompilerParams(vmem_limit_bytes=100 * 1024 * 1024),
    )(A_x.reshape(S, D), A_wqkv, A_wo, B_w1, B_b1, B_w2, B_b2)
    return out.reshape(B, S, D)
```

```python
import functools
import math

import jax
import jax.numpy as jnp
from jax import lax
import jax.experimental.pallas as pl
import jax.experimental.pallas.tpu as pltpu

_H = 32
_EPS = 1e-5
_SB1 = 256
_TQ = 512
_CK = 128
_EXTRA = 2
_NV = 14
_HB = 2
_HP = 2
_DM = 4
_DV = 3
_DK = 3
_QD = 3
_KBSTEPS = (4, 10)
_QSTEPS = (14, 15)
_P3_BOUNDS = (0, 256, 512, 768, 1024, 1280, 1536, 1792, 1984, 2048)
_NI = 4
_B2_OFF = 4096
_PF = 10


def _layernorm(x):
    m = jnp.mean(x, axis=-1, keepdims=True)
    xc = x - m
    v = jnp.mean(xc * xc, axis=-1, keepdims=True)
    return xc * lax.rsqrt(v + _EPS)


def _gelu_tanh(x):
    c = math.sqrt(2.0 / math.pi)
    inner = x * (c + (c * 0.044715) * (x * x))
    hx = 0.5 * x
    return hx + hx * jnp.tanh(inner)


def _kernel(x_hbm, wqkv_hbm, wo_hbm, w1_hbm, b1_hbm, w2_hbm, b2_hbm, o_hbm,
            x_ref, wqkv_ref, wo_ref, w1_ref, w2_ref, o_ref,
            wqvt_scr, kh_scr, qt_scr, vt_scr, ot_scr, s0, s1, s2, s3,
            kb0, kb1, qb_scr, m_scr, l_scr, acc_scr, z_scr, b_ref,
            sems, f_sem,
            *, S, D, F):
    H = _H
    Dh = D // H
    HPG = 128 // Dh
    NG = D // 128
    TQ, CK, SB1 = _TQ, _CK, _SB1
    NQ = S // TQ
    NC = S // CK
    LAG = NC + _EXTRA
    f32 = jnp.float32
    bf16 = jnp.bfloat16
    u32 = jnp.uint32
    qscale = (Dh ** -0.5) * math.log2(math.e)
    sb = [s0, s1, s2, s3]
    kb_scr = [kb0, kb1]
    assert NQ == len(sb)

    XS = 2 * SB1

    def x_copy(i, r0, r1):
        return pltpu.make_async_copy(x_hbm.at[r0:r1, :], x_ref.at[r0:r1, :],
                                     sems.at[3 + i])

    def wqkv_copy(i):
        return pltpu.make_async_copy(wqkv_hbm.at[:, i * D:(i + 1) * D],
                                     wqkv_ref.at[i], sems.at[i])

    HD = D // 2
    wka_copy = pltpu.make_async_copy(wqkv_hbm.at[:, D:D + HD],
                                     wqkv_ref.at[1, :, 0:HD], sems.at[1])
    wkb_copy = pltpu.make_async_copy(wqkv_hbm.at[:, D + HD:2 * D],
                                     wqkv_ref.at[1, :, HD:D], sems.at[6])
    xa_copy = x_copy(0, 0, XS)
    xb_copy = x_copy(1, XS, 2 * XS)
    xc_copy = x_copy(2, 2 * XS, S)
    late_copies = [
        pltpu.make_async_copy(wo_hbm, wo_ref, sems.at[0]),
        pltpu.make_async_copy(w1_hbm, w1_ref, sems.at[0]),
        pltpu.make_async_copy(w2_hbm, w2_ref, sems.at[0]),
        pltpu.make_async_copy(b1_hbm, b_ref.at[0:F], sems.at[0]),
        pltpu.make_async_copy(b2_hbm, b_ref.at[_B2_OFF:_B2_OFF + D], sems.at[0]),
    ]

    def fence():
        pl.semaphore_signal(f_sem, 1)
        pl.semaphore_wait(f_sem, 1)

    for cp in (xa_copy, wka_copy, wkb_copy, wqkv_copy(0), wqkv_copy(2), xb_copy, xc_copy):
        cp.start()
        fence()
    z_scr[...] = jnp.zeros(z_scr.shape, u32)

    N1 = S // SB1
    xn = [None] * N1
    kp = [None] * N1

    def ln1(i):
        xn[i] = _layernorm(x_ref[i * SB1:(i + 1) * SB1, :].astype(f32)).astype(bf16)

    def kmm(i):
        k = jnp.dot(xn[i], wqkv_ref[1], preferred_element_type=f32)
        kp[i] = pltpu.bitcast(k.astype(bf16), u32)

    def khalf(i, n):
        k = jnp.dot(xn[i], wqkv_ref[1, :, n * HD:(n + 1) * HD], preferred_element_type=f32)
        return pltpu.bitcast(k.astype(bf16), u32)

    def kstore(i):
        for g in range(NG):
            kg = kp[i][:, g * 128:(g + 1) * 128]
            for j in range(HPG):
                kr = kg if j == 0 else pltpu.roll(kg, 128 - j * Dh, axis=1)
                kh_scr[g * HPG + j, i * (SB1 // 2):(i + 1) * (SB1 // 2), :] = kr

    def qnat(i):
        q = jnp.dot(xn[i], wqkv_ref[0], preferred_element_type=f32)
        return (q * qscale).astype(bf16)

    def vnat(i):
        v = jnp.dot(xn[i], wqkv_ref[2], preferred_element_type=f32)
        return v.astype(bf16)

    def tstore(dst, i, val):
        dst[:, i * SB1:(i + 1) * SB1] = val.T

    def qvproj(i):
        qv = lax.dot_general(wqvt_scr[...], xn[i], (((1,), (1,)), ((), ())),
                             preferred_element_type=f32)
        qt_scr[:, i * SB1:(i + 1) * SB1] = (qv[0:D] * qscale).astype(bf16)
        vt_scr[:, i * SB1:(i + 1) * SB1] = qv[D:2 * D].astype(bf16)

    xa_copy.wait()
    ln1(0)
    wka_copy.wait()
    ln1(1)
    ka = [khalf(i, 0) for i in range(2)]
    wkb_copy.wait()
    for i in range(2):
        kp[i] = jnp.concatenate([ka[i], khalf(i, 1)], axis=1)
    wqkv_copy(0).wait()
    q0 = qnat(0)
    wqvt_scr[0:D, :] = wqkv_ref[0].T
    q1 = qnat(1)
    tstore(qt_scr, 0, q0)
    wqkv_copy(2).wait()
    xb_copy.wait()
    v0 = vnat(0)
    wqvt_scr[D:2 * D, :] = wqkv_ref[2].T
    v1 = vnat(1)
    ln1(2)
    tstore(qt_scr, 1, q1)
    tstore(vt_scr, 0, v0)
    tstore(vt_scr, 1, v1)
    kstore(0)
    for i in range(2, N1):
        kmm(i)
        if i == 3:
            xc_copy.wait()
        if i + 1 < N1:
            ln1(i + 1)
        qvproj(i)
        kstore(i - 1)
    kstore(N1 - 1)

    T = NQ * NC
    NV = _NV
    KV = 8 * NV
    hi = [KV + (((S - KV) // 16) * (c + 1)) // NC * 16 for c in range(NC)]
    lo = [KV] + hi[:-1]
    assert hi[-1] == S and KV % 16 == 0 and NV <= NC
    NJ = TQ // 128

    def head_rows(h):
        return pl.ds(pl.multiple_of(h * Dh, Dh), Dh)

    def gen_kb(h, kb_ref, ds):
        kf = pltpu.bitcast(kh_scr[h, 0:KV // 2, :], bf16).astype(f32)
        for d in ds:
            kbc = jnp.broadcast_to(kf[:, d:d + 1], (KV, 128))
            kb_ref[d] = kbc
        return kbc[KV - 8:]

    def gen_qb(h, u, ds):
        qf = qt_scr[head_rows(h), (u % NQ) * TQ:(u % NQ + 1) * TQ].astype(f32)
        for d in ds:
            qbc = jnp.broadcast_to(qf[d:d + 1, :], (8, TQ))
            qb_scr[u % qb_scr.shape[0], d] = qbc
        return qbc[:, TQ - 128:]

    def run(h0, n_steps, do1, do2, hook=None, first=False):
        z = jnp.concatenate([z_scr[0:8, :]] * NJ, axis=1)
        m = None
        st = None
        mh = []
        gdep = []
        for t in range(n_steps):
            if do1(t):
                h = h0 + t // T
                u = t // NC
                qb, c = divmod(t % T, NC)
                if first and t == _PF:
                    fence()
                if c in _QSTEPS:
                    n = _QSTEPS.index(c)
                    hq = h0 + (u + 1) // NQ
                    if (u + 1) * NC >= n_steps:
                        hq = jnp.minimum(hq, H - 1)
                    last = gen_qb(hq, u + 1, range(n * Dh // len(_QSTEPS),
                                                   (n + 1) * Dh // len(_QSTEPS)))
                    gdep.append((t + _QD, last))
                kc = pltpu.bitcast(
                    kh_scr[h, pl.ds(lo[c] // 2, (hi[c] - lo[c]) // 2), :],
                    bf16)[:, 0:Dh]
                qt = qt_scr[head_rows(h), qb * TQ:(qb + 1) * TQ]
                s = jnp.dot(kc, qt, preferred_element_type=f32)
                sb[qb][pl.ds(lo[c], hi[c] - lo[c]), :] = s
                mc = jnp.max(s.reshape((hi[c] - lo[c]) // 8, 8, TQ), axis=0)
                m = mc if c == 0 else jnp.maximum(m, mc)
                mh.append(m)
                if c < NV:
                    kbv = kb_scr[(t // T) % 2][:, pl.ds(c * 8, 8), :]
                    if len(mh) >= _DV:
                        depz = pltpu.bitcast(mh[-_DV][:, 0:128], u32) & z[:, 0:128]
                        kbv = pltpu.bitcast(pltpu.bitcast(kbv, u32) | depz[None], f32)
                    acc = jnp.sum(jnp.concatenate([kbv] * NJ, axis=2)
                                  * qb_scr[u % qb_scr.shape[0]], axis=0)
                    sb[qb][pl.ds(c * 8, 8), :] = acc
                    m = jnp.maximum(m, acc)
                if c == NC - 1:
                    m_scr[qb] = jnp.broadcast_to(
                        jnp.max(m, axis=0, keepdims=True), (8, TQ))
                if c in _KBSTEPS:
                    nslot = NQ * len(_KBSTEPS)
                    slot = qb * len(_KBSTEPS) + _KBSTEPS.index(c)
                    last = gen_kb(jnp.minimum(h + 1, H - 1),
                                  kb_scr[(t // T + 1) % 2],
                                  range(slot * Dh // nslot, (slot + 1) * Dh // nslot))
                    gdep.append((t + _DK, last))
                gdep.sort(key=lambda e: e[0])
            t2 = t - LAG
            if do2(t2):
                h2 = h0 + t2 // T
                qb, c = divmod(t2 % T, NC)
                if c == 0:
                    st = (m_scr[qb], jnp.zeros((8, TQ), f32),
                          jnp.zeros((Dh, TQ), f32))
                elif st is None:
                    st = (m_scr[qb], l_scr[...], acc_scr[...])
                mm, l, o = st
                mu = mm
                if len(mh) >= _DM:
                    dep = mh[-_DM]
                    if gdep and t >= gdep[0][0]:
                        dep = jnp.concatenate(
                            [dep[:, 0:128] + gdep.pop(0)[1], dep[:, 128:]], axis=1)
                    mu = pltpu.bitcast(
                        pltpu.bitcast(mm, u32) | (pltpu.bitcast(dep, u32) & z), f32)
                sc = sb[qb][pl.ds(c * CK, CK), :].reshape(CK // 8, 8, TQ)
                p = jnp.exp2(sc - mu[None])
                for i in reversed(range(CK // 16)):
                    l = l + (p[2 * i + 1] + p[2 * i])
                vt = vt_scr[head_rows(h2), pl.ds(c * CK, CK)]
                o = o + jnp.dot(vt, p.reshape(CK, TQ).astype(bf16),
                                preferred_element_type=f32)
                st = (mm, l, o)
                if c == NC - 1:
                    lt = jnp.sum(l, axis=0, keepdims=True)
                    r = pl.reciprocal(lt, approx=True)
                    r = r * (2.0 - lt * r)
                    ot_scr[head_rows(h2), qb * TQ:(qb + 1) * TQ] = (o * r).astype(bf16)
                    st = None
            if hook is not None:
                hook(t)
        if st is not None:
            l_scr[...] = st[1]
            acc_scr[...] = st[2]

    assert (H - _HP) % _HB == 0 and _HP % 2 == 0 and _HB % 2 == 0
    gen_kb(0, kb_scr[0], range(Dh))
    gen_qb(0, 0, range(Dh))
    run(0, _HP * T, lambda t: True, lambda t2: t2 >= 0, first=True)
    for cp in late_copies:
        cp.start()

    def body(i, carry):
        run(_HP + i * _HB, _HB * T, lambda t: True, lambda t2: True)
        return carry

    lax.fori_loop(0, (H - _HP) // _HB, body, 0)
    for cp in late_copies:
        cp.wait()

    bounds = _P3_BOUNDS
    NS = len(bounds) - 1
    rows = [pl.ds(bounds[i], bounds[i + 1] - bounds[i]) for i in range(NS)]
    hs = [None] * NS
    gs = [None] * NS
    b1 = b_ref[0:F].astype(f32).reshape(1, F)
    b2 = b_ref[_B2_OFF:_B2_OFF + D].astype(f32).reshape(1, D)

    def o_copy(i):
        return pltpu.make_async_copy(o_ref.at[rows[i], :], o_hbm.at[rows[i], :],
                                     sems.at[1])

    def op(i):
        attn = lax.dot_general(ot_scr[:, rows[i]], wo_ref[...],
                               (((0,), (0,)), ((), ())),
                               preferred_element_type=f32)
        hs[i] = x_ref[rows[i], :].astype(f32) + attn

    def f1(i, hn=None):
        if hn is None:
            hn = _layernorm(hs[i]).astype(bf16)
        a = jnp.dot(hn, w1_ref[...], preferred_element_type=f32)
        gs[i] = _gelu_tanh(a + b1).astype(bf16)

    def f2(i):
        y = jnp.dot(gs[i], w2_ref[...], preferred_element_type=f32)
        o_ref[rows[i], :] = (hs[i] + (y + b2)).astype(o_ref.dtype)
        o_copy(i).start()

    NI = _NI
    assert bounds[NI] <= ((T - LAG) // NC) * TQ
    pieces = {}
    ob = [ot_scr[:, rows[i]].T for i in range(NI)]

    def hook(t):
        for _ in range(((t + 1) * NI * NG) // LAG - len(pieces)):
            i, g = divmod(len(pieces), NG)
            pieces[(i, g)] = jnp.dot(ob[i], wo_ref[:, g * 128:(g + 1) * 128],
                                     preferred_element_type=f32)

    run(H, LAG, lambda t: False, lambda t2: True, hook)
    for i in range(NI):
        attn = jnp.concatenate([pieces[(i, g)] for g in range(NG)], axis=1)
        hs[i] = x_ref[rows[i], :].astype(f32) + attn
    hn0 = _layernorm(hs[0]).astype(bf16)
    fence()
    for i in range(NS):
        f1(i, hn0 if i == 0 else None)
        if NI <= i + 2 < NS:
            op(i + 2)
        if i >= 1:
            f2(i - 1)
    f2(NS - 1)
    for i in range(NS):
        o_copy(i).wait()


@jax.jit
def pallas_sequential_preLN__softmax_full_mha__dense_activation_gelu__prompt_kernel(
    A_x: jax.Array,
    A_wqkv: jax.Array,
    A_wo: jax.Array,
    B_x: jax.Array,
    B_w1: jax.Array,
    B_b1: jax.Array,
    B_w2: jax.Array,
    B_b2: jax.Array,
):
    del B_x
    B, S, D = A_x.shape
    F = B_w1.shape[1]
    assert B == 1 and S == _P3_BOUNDS[-1] and F <= _B2_OFF
    bf16 = jnp.bfloat16
    f32 = jnp.float32
    nq = S // _TQ
    dh = D // _H
    hbm = pl.BlockSpec(memory_space=pl.ANY)
    out = pl.pallas_call(
        functools.partial(_kernel, S=S, D=D, F=F),
        out_shape=jax.ShapeDtypeStruct((S, D), A_x.dtype),
        in_specs=[hbm] * 7,
        out_specs=hbm,
        scratch_shapes=[
            pltpu.VMEM((S, D), bf16),
            pltpu.VMEM((3, D, D), bf16),
            pltpu.VMEM((D, D), bf16),
            pltpu.VMEM((D, F), bf16),
            pltpu.VMEM((F, D), bf16),
            pltpu.VMEM((S, D), A_x.dtype),
            pltpu.VMEM((2 * D, D), bf16),
            pltpu.VMEM((_H, S // 2, 128), jnp.uint32),
            pltpu.VMEM((D, S), bf16),
            pltpu.VMEM((D, S), bf16),
            pltpu.VMEM((D, S), bf16),
        ] + [pltpu.VMEM((S, _TQ), f32)] * nq + [
            pltpu.VMEM((dh, 8 * _NV, 128), f32),
            pltpu.VMEM((dh, 8 * _NV, 128), f32),
            pltpu.VMEM((_HB * nq, dh, 8, _TQ), f32),
            pltpu.VMEM((nq, 8, _TQ), f32),
            pltpu.VMEM((8, _TQ), f32),
            pltpu.VMEM((dh, _TQ), f32),
            pltpu.VMEM((32, 128), jnp.uint32),
            pltpu.VMEM((2 * _B2_OFF,), bf16),
            pltpu.SemaphoreType.DMA((7,)),
            pltpu.SemaphoreType.REGULAR,
        ],
        compiler_params=pltpu.CompilerParams(vmem_limit_bytes=100 * 1024 * 1024),
    )(A_x.reshape(S, D), A_wqkv, A_wo, B_w1, B_b1, B_w2, B_b2)
    return out.reshape(B, S, D)
```
